```python
import os as _os
_os.environ.setdefault("JAX_PLATFORMS", "cpu")
import jax
import jax.numpy as jnp

def _softmax(x, axis=-1):
    return jax.nn.softmax(x, axis=axis)
def _gelu(x):
    return jax.nn.gelu(x, approximate=True)
def _silu(x):
    return jax.nn.silu(x)
def _sigmoid(x):
    return jax.nn.sigmoid(x)
def _layernorm(x, axis=-1, eps=1e-5):
    m = jnp.mean(x, axis=axis, keepdims=True)
    v = jnp.var(x, axis=axis, keepdims=True)
    return (x - m) / jnp.sqrt(v + eps)
def _scatter_add(tgt, idx, src, axis=0):
    return tgt.at[idx].add(src)
def _segment_sum(src, seg, n):
    return jax.ops.segment_sum(src, seg, n)
class _Rng:
    def __init__(self, key):
        self._k = key
    def _next(self):
        self._k, sub = jax.random.split(self._k)
        return sub
    def normal(self, shape):
        return jax.random.normal(self._next(), shape, dtype=jnp.bfloat16)
    def randint(self, lo, hi, shape):
        return jax.random.randint(self._next(), shape, lo, hi, dtype=jnp.int32)
    def uniform(self, shape, lo=0.0, hi=1.0):
        return jax.random.uniform(self._next(), shape, jnp.bfloat16, lo, hi)
    def permutation(self, n):
        return jax.random.permutation(self._next(), n)


kernel_name = 'interleave_layers__linear_attn_block__mha_block__prompt'

def setup_inputs():
    _rng = _Rng(jax.random.key(int.from_bytes(__import__("os").urandom(4), "little")))
    _w = (lambda a: (lambda t: t.astype(jnp.bfloat16) if jnp.issubdtype(t.dtype, jnp.floating) else t)(jnp.asarray(a)))
    def _A_setup():
        B, S, D = 1, 2048, 640
        return {
            "x": _w((lambda *s: _rng.normal(s) * 0.05)(B, S, D)),
            "wqkv": _w((lambda *s: _rng.normal(s) * 0.1)(D, 3 * D)),
            "wo": _w((lambda *s: _rng.normal(s) * 0.05)(D, D)),
        }
    _A_in = _A_setup()

    def _B_setup():
        B, S, D, H = 1, 2048, 640, 32
        return {
            "x": _w((lambda *s: _rng.normal(s) * 0.05)(B, S, D)),
            "wqkv": _w((lambda *s: _rng.normal(s) * 0.1)(D, 3 * D)),
            "wo": _w((lambda *s: _rng.normal(s) * 0.05)(D, D)),
        }
    _B_in = _B_setup()

    return {
        "A_x": _A_in["x"],
        "A_wqkv": _A_in["wqkv"],
        "A_wo": _A_in["wo"],
        "B_x": _B_in["x"],
        "B_wqkv": _B_in["wqkv"],
        "B_wo": _B_in["wo"],
    }

def reference(A_x, A_wqkv, A_wo, B_x, B_wqkv, B_wo):
    def _A_ref(x, wqkv, wo):
        B, S, D = x.shape
        H = 32; Dh = D // H
        qkv = (lambda x, *d: x.transpose(*d))((x @ wqkv).reshape(B, S, 3, H, Dh), 2, 0, 3, 1, 4)
        q, k, v = qkv[0], qkv[1], qkv[2]
        phi = lambda t: jnp.where(t > 0, t + 1, jnp.exp(t)) + 1e-6
        pq, pk = phi(q), phi(k)
        kv = jnp.einsum("bhsd,bhse->bhde", pk, v)
        z = jnp.einsum("bhsd->bhd", pk)
        num = jnp.einsum("bhqd,bhde->bhqe", pq, kv)
        den = jnp.einsum("bhqd,bhd->bhq", pq, z)[..., None] + 1e-6
        o = num / den
        return (lambda x, *d: x.transpose(*d))(o, 0, 2, 1, 3).reshape(B, S, D) @ wo

    def _B_ref(x, wqkv, wo):
        B, S, D = x.shape
        H = 32
        Dh = D // H
        qkv = (lambda x, *d: x.transpose(*d))((x @ wqkv).reshape(B, S, 3, H, Dh), 2, 0, 3, 1, 4)
        q, k, v = qkv[0], qkv[1], qkv[2]
        scores = jnp.einsum("bhqd,bhkd->bhqk", q, k) * (Dh ** -0.5)
        p = _softmax(scores, axis=-1)
        o = jnp.einsum("bhqk,bhkd->bhqd", p, v)
        return (lambda x, *d: x.transpose(*d))(o, 0, 2, 1, 3).reshape(B, S, D) @ wo

    x = A_x
    x = x + _A_ref(_layernorm(x, axis=-1), A_wqkv, A_wo)
    x = x + _B_ref(_layernorm(x, axis=-1), B_wqkv, B_wo)
    x = x + _A_ref(_layernorm(x, axis=-1), A_wqkv, A_wo)
    x = x + _B_ref(_layernorm(x, axis=-1), B_wqkv, B_wo)
    return x
```

```python
import math

import jax
import jax.numpy as jnp
from jax import lax
import jax.experimental.pallas as pl
import jax.experimental.pallas.tpu as pltpu

S = 2048
D = 640
H = 32
DH = D // H
LANES = 128
NT_D = D // LANES
TB = 256
TQ = 512
CK = 128
VW = 24
Q_SCALE = DH ** -0.5 * math.log2(math.e)

F32 = jnp.float32
BF16 = jnp.bfloat16

NN = (((1,), (0,)), ((), ()))
NT = (((1,), (1,)), ((), ()))
TN = (((0,), (0,)), ((), ()))


def _dot(a, b, dims=NN):
    return lax.dot_general(a, b, dims, preferred_element_type=F32)


def _band(e):
    lo = (LANES * e) // DH * DH
    hi = -(-(LANES * (e + 1)) // DH) * DH
    return lo // 8 * 8, -(-hi // 8) * 8


BANDS = [_band(e) for e in range(NT_D)]
BAND_MAX = max(hi - lo for lo, hi in BANDS)


def _layernorm(x):
    m = jnp.mean(x, axis=-1, keepdims=True)
    c = x - m
    v = jnp.mean(c * c, axis=-1, keepdims=True)
    return (c * lax.rsqrt(v + 1e-5)).astype(BF16)


def _phi(t):
    return jnp.where(t > 0, t + 1, jnp.exp(t)) + 1e-6


def _head_of(i):
    return (i * 3277) >> 16


def _straddlers(w_ref, col0):
    parts = []
    for b in range(NT_D - 1):
        lo = col0 + (LANES * (b + 1)) // DH * DH
        parts.append(w_ref[:, lo:lo + DH].astype(F32))
        parts.append(jnp.zeros((D, 32 - DH), F32))
    return jnp.concatenate(parts, axis=1)


def _kernel(x_ref, awqkv, awo, bwqkv, bwo, out_ref,
            xs, awkT, bwqvT, bwk_x, pq, kv_acc, z_acc, m_acc, mw, zexp,
            ks, qs, vts, ots, s_scr, m_scr, vm):
    awkT[...] = awqkv[:, D:2 * D].astype(F32).T.astype(BF16)
    bwqvT[0:D, :] = bwqkv[:, 0:D].astype(F32).T.astype(BF16)
    bwqvT[D:D + LANES, :] = _straddlers(bwqkv, 0).T.astype(BF16)
    bwqvT[D + LANES:, :] = bwqkv[:, 2 * D:3 * D].astype(F32).T.astype(BF16)
    bwk_x[...] = _straddlers(bwqkv, D).astype(BF16)

    def rows(j):
        return pl.ds(pl.multiple_of(j * TB, TB), TB)

    def a_proj(j, xb):
        xn = _layernorm(xb)
        pq[rows(j), :] = _phi(_dot(xn, awqkv[:, 0:D])).astype(BF16)
        v = _dot(xn, awqkv[:, 2 * D:3 * D]).astype(BF16)
        pk = _phi(_dot(awkT[...], xn, NT))
        z = z_acc[...]
        for t in range(TB // LANES):
            z = z + pk[:, t * LANES:(t + 1) * LANES]
        z_acc[...] = z
        for e, (lo, hi) in enumerate(BANDS):
            kv_acc[e, 0:hi - lo, :] += _dot(pk[lo:hi, :], v[:, e * LANES:(e + 1) * LANES])

    def a_reduce():
        z = jnp.sum(z_acc[...], axis=-1, keepdims=True)
        m_acc[...] = jnp.zeros_like(m_acc)
        for e, (lo, hi) in enumerate(BANDS):
            r = lax.broadcasted_iota(jnp.int32, (D, LANES), 0)
            c = lax.broadcasted_iota(jnp.int32, (D, LANES), 1) + e * LANES
            same = _head_of(r) == _head_of(c)
            zexp[:, e * LANES:(e + 1) * LANES] = jnp.where(same, z, 0.0).astype(BF16)
            kv = jnp.where(same[lo:hi, :], kv_acc[e, 0:hi - lo, :], 0.0)
            m_acc[lo:hi, :] += _dot(kv, awo[e * LANES:(e + 1) * LANES, :])
        mw[...] = m_acc[...].astype(BF16)

    def a_out(j):
        p = pq[rows(j), :]
        parts = []
        for e in range(NT_D):
            lo, hi = max(e - 1, 0) * LANES, min(e + 2, NT_D) * LANES
            den = _dot(p[:, lo:hi], zexp[lo:hi, e * LANES:(e + 1) * LANES]) + 1e-6
            parts.append((p[:, e * LANES:(e + 1) * LANES].astype(F32) / den).astype(BF16))
        xb = xs[rows(j), :] + _dot(jnp.concatenate(parts, axis=1), mw[...])
        xs[rows(j), :] = xb
        return xb

    def b_proj(j, xb):
        xn = _layernorm(xb)
        k = _dot(xn, bwqkv[:, D:2 * D]).astype(BF16)
        for t in range(NT_D):
            ks[t, rows(j), :] = k[:, t * LANES:(t + 1) * LANES]
        ks[NT_D, rows(j), :] = _dot(xn, bwk_x[...]).astype(BF16)
        qv = _dot(bwqvT[...], xn, NT)
        for t in range(NT_D + 1):
            qs[t, :, rows(j)] = (qv[t * LANES:(t + 1) * LANES, :] * Q_SCALE).astype(BF16)
        vts[:, rows(j)] = qv[D + LANES:, :]

    def head_q(h, t):
        blk = (h * DH) // LANES
        off = h * DH - blk * LANES
        cross = off + DH > LANES
        off = jnp.where(cross, blk * 32, off)
        blk = jnp.where(cross, NT_D, blk)
        r = lax.broadcasted_iota(jnp.int32, (LANES, TQ), 0)
        q = qs[blk, :, t * TQ:(t + 1) * TQ].astype(F32)
        return blk, jnp.where((r >= off) & (r < off + DH), q, 0.0).astype(BF16)

    def attn_step(h_qk, h_pv):
        if h_pv is not None:
            r0 = pl.multiple_of((h_pv * DH) // 8 * 8, 8)
            o0 = h_pv * DH - r0
            r = lax.broadcasted_iota(jnp.int32, (VW, S), 0)
            vm[...] = jnp.where((r >= o0) & (r < o0 + DH), vts[pl.ds(r0, VW), :], 1.0)
        for t in range(S // TQ):
            cols = slice(t * TQ, (t + 1) * TQ)
            if h_qk is not None:
                blk, q = head_q(h_qk, t)
            if h_pv is not None:
                m_old = m_scr[0:1, cols]
            m = acc = None
            for c in range(S // CK):
                keys = slice(c * CK, (c + 1) * CK)
                if h_qk is not None:
                    st = _dot(ks[blk, keys, :], q)
                if h_pv is not None:
                    old = s_scr[t, keys, :]
                if h_qk is not None:
                    s_scr[t, keys, :] = st
                    mm = jnp.max(st.reshape(CK // 8, 8, TQ), axis=0)
                    m = mm if m is None else jnp.maximum(m, mm)
                if h_pv is not None:
                    p = jnp.exp2(old - m_old).astype(BF16)
                    o = _dot(vm[:, keys], p)
                    acc = o if acc is None else acc + o
            if h_pv is not None:
                den = jnp.where(o0 == 0, acc[VW - 1:VW, :], acc[0:1, :])
                r = lax.broadcasted_iota(jnp.int32, (VW, TQ), 0)
                ots[pl.ds(r0, VW), cols] = jnp.where(r >= o0, acc / den, ots[pl.ds(r0, VW), cols])
            if h_qk is not None:
                m_scr[:, cols] = jnp.broadcast_to(jnp.max(m, axis=0, keepdims=True), (8, TQ))

    def b_out(j):
        o = ots[:, rows(j)].astype(BF16)
        return xs[rows(j), :] + _dot(o, bwo[...], TN)

    def for_blocks(fn):
        def body(j, carry):
            fn(j)
            return carry
        lax.fori_loop(0, S // TB, body, 0)

    def layer_pair(layer, carry):
        z_acc[...] = jnp.zeros_like(z_acc)
        kv_acc[...] = jnp.zeros_like(kv_acc)

        @pl.when(layer == 0)
        def _():
            def first(j):
                xb = x_ref[rows(j), :].astype(F32)
                xs[rows(j), :] = xb
                a_proj(j, xb)
            for_blocks(first)

        @pl.when(layer != 0)
        def _():
            def later(j):
                xb = b_out(j)
                xs[rows(j), :] = xb
                a_proj(j, xb)
            for_blocks(later)

        a_reduce()
        for_blocks(lambda j: b_proj(j, a_out(j)))

        attn_step(0, None)

        def head_body(h, c):
            attn_step(h, h - 1)
            return c
        lax.fori_loop(1, H, head_body, 0)
        attn_step(None, H - 1)
        return carry

    lax.fori_loop(0, 2, layer_pair, 0)

    def last(j):
        out_ref[rows(j), :] = b_out(j).astype(out_ref.dtype)
    for_blocks(last)


@jax.jit
def pallas_interleave_layers__linear_attn_block__mha_block__prompt_kernel(
    A_x: jax.Array,
    A_wqkv: jax.Array,
    A_wo: jax.Array,
    B_x: jax.Array,
    B_wqkv: jax.Array,
    B_wo: jax.Array,
):
    del B_x
    out = pl.pallas_call(
        _kernel,
        out_shape=jax.ShapeDtypeStruct((S, D), A_x.dtype),
        scratch_shapes=[
            pltpu.VMEM((S, D), F32),
            pltpu.VMEM((D, D), BF16),
            pltpu.VMEM((2 * D + LANES, D), BF16),
            pltpu.VMEM((D, LANES), BF16),
            pltpu.VMEM((S, D), BF16),
            pltpu.VMEM((NT_D, BAND_MAX, LANES), F32),
            pltpu.VMEM((D, LANES), F32),
            pltpu.VMEM((D, D), F32),
            pltpu.VMEM((D, D), BF16),
            pltpu.VMEM((D, D), BF16),
            pltpu.VMEM((NT_D + 1, S, LANES), BF16),
            pltpu.VMEM((NT_D + 1, LANES, S), BF16),
            pltpu.VMEM((D, S), F32),
            pltpu.VMEM((D, S), F32),
            pltpu.VMEM((S // TQ, S, TQ), F32),
            pltpu.VMEM((8, S), F32),
            pltpu.VMEM((VW, S), F32),
        ],
        compiler_params=pltpu.CompilerParams(vmem_limit_bytes=100 * 1024 * 1024),
    )(A_x.reshape(S, D), A_wqkv, A_wo, B_wqkv, B_wo)
    return out.reshape(A_x.shape)
```

```python
import math

import jax
import jax.numpy as jnp
from jax import lax
import jax.experimental.pallas as pl
import jax.experimental.pallas.tpu as pltpu

S = 2048
D = 640
H = 32
DH = D // H
LANES = 128
ND = D // LANES
TB = 256
NSUB = 2
TQ = 512
CK = 128
VW = 24
Q_SCALE = DH ** -0.5 * math.log2(math.e)

F32 = jnp.float32
BF16 = jnp.bfloat16

NN = (((1,), (0,)), ((), ()))
NT = (((1,), (1,)), ((), ()))
TN = (((0,), (0,)), ((), ()))


def _dot(a, b, dims=NN):
    return lax.dot_general(a, b, dims, preferred_element_type=F32)


def _tile(e):
    return slice(e * LANES, (e + 1) * LANES)


def _band(e):
    lo = (LANES * e) // DH * DH
    hi = -(-(LANES * (e + 1)) // DH) * DH
    return lo // 8 * 8, -(-hi // 8) * 8


BANDS = [_band(e) for e in range(ND)]
BAND_MAX = max(hi - lo for lo, hi in BANDS)


def _layernorm(x):
    m = jnp.mean(x, axis=-1, keepdims=True)
    c = x - m
    v = jnp.mean(c * c, axis=-1, keepdims=True)
    return (c * lax.rsqrt(v + 1e-5)).astype(BF16)


def _phi(t):
    return jnp.where(t > 0, t + 1, jnp.exp(t)) + 1e-6


def _head_of(i):
    return (i * 3277) >> 16


def _kernel(x_hbm, awqkv_hbm, awo_hbm, bwqkv_hbm, bwo_hbm, out_hbm,
            io, awqkv, awo, bwqkv, bwo, x_sem, w_sem,
            xs, awqkT, bwqvT, pqT, g_acc, z_acc, m_acc, mw, zh,
            ks, qs, vts, ots, s_scr, m_scr, vm):
    blk = TB * NSUB

    def x_copy(j):
        r = pl.ds(pl.multiple_of(j * blk, blk), blk)
        return pltpu.make_async_copy(x_hbm.at[r, :], io.at[r, :], x_sem.at[j])

    def out_copy(j):
        r = pl.ds(pl.multiple_of(j * blk, blk), blk)
        return pltpu.make_async_copy(io.at[r, :], out_hbm.at[r, :], x_sem.at[j])

    def col_copy(src, dst, part, sem):
        c = slice(part * D, (part + 1) * D)
        return pltpu.make_async_copy(src.at[:, c], dst.at[:, c], w_sem.at[sem])

    aw_copies = [col_copy(awqkv_hbm, awqkv, part, part) for part in (1, 0, 2)]
    awo_copy = pltpu.make_async_copy(awo_hbm, awo, w_sem.at[3])
    bwqkv_copy = pltpu.make_async_copy(bwqkv_hbm, bwqkv, w_sem.at[4])
    bwo_copy = pltpu.make_async_copy(bwo_hbm, bwo, w_sem.at[5])

    with jax.named_scope("prep"):
        aw_copies[0].start()
        aw_copies[1].start()
        x_copy(0).start()
        aw_copies[0].wait()
        awqkT[D:, :] = awqkv[:, D:2 * D].astype(F32).T.astype(BF16)
        aw_copies[1].wait()
        for j in range(1, S // blk):
            x_copy(j).start()
        awqkT[0:D, :] = awqkv[:, 0:D].astype(F32).T.astype(BF16)
        aw_copies[2].start()
        awo_copy.start()
        bwqkv_copy.start()
        bwo_copy.start()

    upper = lax.broadcasted_iota(jnp.int32, (TB, LANES), 1) >= LANES // 2

    def for_blocks(fn, before=None, after=None):
        def body(j, carry):
            if before is not None:
                before(j)
            fn([pl.ds(pl.multiple_of((j * NSUB + u) * TB, TB), TB) for u in range(NSUB)])
            if after is not None:
                after(j)
            return carry
        lax.fori_loop(0, S // (TB * NSUB), body, 0)

    def a_proj(rows, xbs):
        xns = [_layernorm(xb) for xb in xbs]
        pks = []
        for r, xn in zip(rows, xns):
            qk = _phi(_dot(awqkT[...], xn, NT))
            pqT[:, r] = qk[0:D].astype(BF16)
            pks.append(qk[D:])
        pk = jnp.concatenate(pks, axis=1)
        z = z_acc[...]
        for t in range(TB * NSUB // LANES):
            z = z + pk[:, _tile(t)]
        z_acc[...] = z
        g_acc[...] += _dot(pk, jnp.concatenate(xns, axis=0))

    def a_reduce():
        z = jnp.sum(z_acc[...].T, axis=0, keepdims=True)
        h = lax.broadcasted_iota(jnp.int32, (H, D), 0)
        d = lax.broadcasted_iota(jnp.int32, (H, D), 1)
        zh[...] = jnp.where(_head_of(d) == h, z, 0.0)
        m_acc[...] = jnp.zeros_like(m_acc)
        for e, (lo, hi) in enumerate(BANDS):
            r = lax.broadcasted_iota(jnp.int32, (hi - lo, LANES), 0) + lo
            c = lax.broadcasted_iota(jnp.int32, (hi - lo, LANES), 1) + e * LANES
            kv = _dot(g_acc[lo:hi, :], awqkv[:, 2 * D + e * LANES:2 * D + (e + 1) * LANES])
            kv = jnp.where(_head_of(r) == _head_of(c), kv, 0.0)
            m_acc[lo:hi, :] += _dot(kv, awo[_tile(e), :])
        mw[...] = m_acc[...].astype(BF16)

    def a_out(rows):
        low = lax.broadcasted_iota(jnp.int32, (8, TB), 0) < 4
        ratios = []
        for r in rows:
            p = pqT[:, r]
            inv = 1.0 / (_dot(zh[...], p) + 1e-6)
            parts = []
            for h in range(0, H, 2):
                a = jnp.broadcast_to(inv[h:h + 1], (8, TB))
                b = jnp.broadcast_to(inv[h + 1:h + 2], (8, TB))
                parts += [a, a, jnp.where(low, a, b), b, b]
            ratios.append((p.astype(F32) * jnp.concatenate(parts, axis=0)).astype(BF16))
        xbs = []
        for r, ratio in zip(rows, ratios):
            xb = xs[r, :] + _dot(ratio, mw[...], TN)
            xs[r, :] = xb
            xbs.append(xb)
        return xbs

    def b_proj(rows, xbs):
        for r, xb in zip(rows, xbs):
            xn = _layernorm(xb)
            k = _dot(xn, bwqkv[:, D:2 * D]).astype(BF16)
            for t in range(ND):
                ks[t, r, :] = k[:, _tile(t)]
            for t in range(ND - 1):
                ks[ND + t, r, :] = jnp.where(upper, k[:, _tile(t)], k[:, _tile(t + 1)])
            qv = _dot(bwqvT[...], xn, NT)
            for t in range(ND):
                qs[t, :, r] = (qv[_tile(t), :] * Q_SCALE).astype(BF16)
            vts[:, r] = qv[D:, :]

    def head_q(h, t):
        blk = (h * DH) // LANES
        off = h * DH - blk * LANES
        cross = jnp.where(off + DH > LANES, 1, 0)
        cols = slice(t * TQ, (t + 1) * TQ)
        half = LANES // 2
        q = jnp.concatenate([qs[blk + cross, 0:half, cols], qs[blk, half:, cols]], axis=0)
        r = lax.broadcasted_iota(jnp.int32, (LANES, TQ), 0)
        mine = ((r - off) & (LANES - 1)) < DH
        return blk + ND * cross, jnp.where(mine, q.astype(F32), 0.0).astype(BF16)

    def attn_step(h_qk, h_pv):
        if h_pv is not None:
            r0 = pl.multiple_of((h_pv * DH) // 8 * 8, 8)
            o0 = h_pv * DH - r0
            r = lax.broadcasted_iota(jnp.int32, (VW, S), 0)
            vm[...] = jnp.where((r >= o0) & (r < o0 + DH), vts[pl.ds(r0, VW), :], 1.0)
        for t in range(S // TQ):
            cols = slice(t * TQ, (t + 1) * TQ)
            if h_qk is not None:
                blk, q = head_q(h_qk, t)
            if h_pv is not None:
                m_old = m_scr[0:1, cols]
            m = acc = None
            for c in range(S // CK):
                keys = slice(c * CK, (c + 1) * CK)
                if h_qk is not None:
                    st = _dot(ks[blk, keys, :], q)
                if h_pv is not None:
                    old = s_scr[t, keys, :]
                if h_qk is not None:
                    s_scr[t, keys, :] = st
                    mm = jnp.max(st.reshape(CK // 8, 8, TQ), axis=0)
                    m = mm if m is None else jnp.maximum(m, mm)
                if h_pv is not None:
                    p = jnp.exp2(old - m_old).astype(BF16)
                    o = _dot(vm[:, keys], p)
                    acc = o if acc is None else acc + o
            if h_pv is not None:
                den = jnp.where(o0 == 0, acc[VW - 1:VW, :], acc[0:1, :])
                r = lax.broadcasted_iota(jnp.int32, (VW, TQ), 0)
                ots[pl.ds(r0, VW), cols] = jnp.where(r >= o0, acc / den, ots[pl.ds(r0, VW), cols])
            if h_qk is not None:
                m_scr[:, cols] = jnp.broadcast_to(jnp.max(m, axis=0, keepdims=True), (8, TQ))

    def b_out(rows):
        return [xs[r, :] + _dot(ots[:, r].astype(BF16), bwo[...], TN) for r in rows]

    def layer_pair(layer, carry):
        z_acc[...] = jnp.zeros_like(z_acc)
        g_acc[...] = jnp.zeros_like(g_acc)

        @pl.when(layer == 0)
        def _():
            def first(rows):
                xbs = [io[r, :].astype(F32) for r in rows]
                for r, xb in zip(rows, xbs):
                    xs[r, :] = xb
                a_proj(rows, xbs)
            with jax.named_scope("first"):
                for_blocks(first, before=lambda j: x_copy(j).wait())
            with jax.named_scope("prep2"):
                aw_copies[2].wait()
                awo_copy.wait()
                bwqkv_copy.wait()
                bwo_copy.wait()
                bwqvT[0:D, :] = bwqkv[:, 0:D].astype(F32).T.astype(BF16)
                bwqvT[D:, :] = bwqkv[:, 2 * D:3 * D].astype(F32).T.astype(BF16)

        @pl.when(layer != 0)
        def _():
            def later(rows):
                xbs = b_out(rows)
                for r, xb in zip(rows, xbs):
                    xs[r, :] = xb
                a_proj(rows, xbs)
            with jax.named_scope("later"):
                for_blocks(later)

        with jax.named_scope("a_reduce"):
            a_reduce()
        with jax.named_scope("aout_bproj"):
            for_blocks(lambda rows: b_proj(rows, a_out(rows)))

        with jax.named_scope("attn_pro"):
            attn_step(0, None)

        def head_body(h, c):
            attn_step(h, h - 1)
            return c
        with jax.named_scope("attn_main"):
            lax.fori_loop(1, H, head_body, 0)
        with jax.named_scope("attn_epi"):
            attn_step(None, H - 1)
        return carry

    lax.fori_loop(0, 2, layer_pair, 0)

    def last(rows):
        for r, xb in zip(rows, b_out(rows)):
            io[r, :] = xb.astype(io.dtype)
    with jax.named_scope("last"):
        for_blocks(last, after=lambda j: out_copy(j).start())
        for j in range(S // blk):
            out_copy(j).wait()


@jax.jit
def pallas_interleave_layers__linear_attn_block__mha_block__prompt_kernel(
    A_x: jax.Array,
    A_wqkv: jax.Array,
    A_wo: jax.Array,
    B_x: jax.Array,
    B_wqkv: jax.Array,
    B_wo: jax.Array,
):
    del B_x
    out = pl.pallas_call(
        _kernel,
        out_shape=jax.ShapeDtypeStruct((S, D), A_x.dtype),
        in_specs=[pl.BlockSpec(memory_space=pl.ANY)] * 5,
        out_specs=pl.BlockSpec(memory_space=pl.ANY),
        scratch_shapes=[
            pltpu.VMEM((S, D), BF16),
            pltpu.VMEM((D, 3 * D), BF16),
            pltpu.VMEM((D, D), BF16),
            pltpu.VMEM((D, 3 * D), BF16),
            pltpu.VMEM((D, D), BF16),
            pltpu.SemaphoreType.DMA((S // (TB * NSUB),)),
            pltpu.SemaphoreType.DMA((6,)),
            pltpu.VMEM((S, D), F32),
            pltpu.VMEM((2 * D, D), BF16),
            pltpu.VMEM((2 * D, D), BF16),
            pltpu.VMEM((D, S), BF16),
            pltpu.VMEM((D, D), F32),
            pltpu.VMEM((D, LANES), F32),
            pltpu.VMEM((D, D), F32),
            pltpu.VMEM((D, D), BF16),
            pltpu.VMEM((H, D), F32),
            pltpu.VMEM((2 * ND - 1, S, LANES), BF16),
            pltpu.VMEM((ND, LANES, S), BF16),
            pltpu.VMEM((D, S), F32),
            pltpu.VMEM((D, S), F32),
            pltpu.VMEM((S // TQ, S, TQ), F32),
            pltpu.VMEM((8, S), F32),
            pltpu.VMEM((VW, S), F32),
        ],
        compiler_params=pltpu.CompilerParams(vmem_limit_bytes=100 * 1024 * 1024),
    )(A_x.reshape(S, D), A_wqkv, A_wo, B_wqkv, B_wo)
    return out.reshape(A_x.shape)
```

```python
import math

import jax
import jax.numpy as jnp
from jax import lax
import jax.experimental.pallas as pl
import jax.experimental.pallas.tpu as pltpu

S = 2048
D = 640
H = 32
DH = D // H
LANES = 128
HALF = LANES // 2
ND = D // LANES
TB = 256
NSUB = 2
BLK = TB * NSUB
NBLK = S // BLK
CK = 128
VW = 24
Q_SCALE = DH ** -0.5 * math.log2(math.e)

F32 = jnp.float32
BF16 = jnp.bfloat16

NN = (((1,), (0,)), ((), ()))
NT = (((1,), (1,)), ((), ()))
TN = (((0,), (0,)), ((), ()))


def _dot(a, b, dims=NN):
    return lax.dot_general(a, b, dims, preferred_element_type=F32)


def _tile(e):
    return slice(e * LANES, (e + 1) * LANES)


def _band(e):
    lo = (LANES * e) // DH * DH
    hi = -(-(LANES * (e + 1)) // DH) * DH
    return lo // 8 * 8, -(-hi // 8) * 8


def _span(i, n):
    return pl.ds(pl.multiple_of(i * n, n), n)


def _loop(lo, hi, fn):
    def body(i, carry):
        fn(i)
        return carry
    lax.fori_loop(lo, hi, body, 0)


def _iota(shape, dim):
    return lax.broadcasted_iota(jnp.int32, shape, dim)


def _layernorm(x):
    c = x - jnp.mean(x, axis=-1, keepdims=True)
    v = jnp.mean(c * c, axis=-1, keepdims=True)
    return (c * lax.rsqrt(v + 1e-5)).astype(BF16)


def _phi(t):
    return jnp.where(t > 0, t + 1, jnp.exp(t)) + 1e-6


def _head_of(i):
    return (i * 3277) >> 16


def _transposed(w):
    return w.astype(F32).T.astype(BF16)


def _kernel(x_hbm, awqkv_hbm, awo_hbm, bwqkv_hbm, bwo_hbm, out_hbm,
            io, awqkv, awo, bwqkv, bwo, x_sem, w_sem,
            xs, xns, awqkT, bwqvT, pqT, g_acc, z_acc, m_acc, mw, zh,
            ks, qs, vts, ots, s_scr, m_scr, vm):
    def x_copy(j):
        return pltpu.make_async_copy(x_hbm.at[_span(j, BLK), :], io.at[_span(j, BLK), :], x_sem.at[j])

    def out_copy(j):
        return pltpu.make_async_copy(io.at[_span(j, BLK), :], out_hbm.at[_span(j, BLK), :], x_sem.at[j])

    def a_part_copy(part):
        c = slice(part * D, (part + 1) * D)
        return pltpu.make_async_copy(awqkv_hbm.at[:, c], awqkv.at[:, c], w_sem.at[part])

    awq_copy, awk_copy, awv_copy = (a_part_copy(p) for p in range(3))
    late_copies = [
        awv_copy,
        pltpu.make_async_copy(awo_hbm, awo, w_sem.at[3]),
        pltpu.make_async_copy(bwqkv_hbm, bwqkv, w_sem.at[4]),
        pltpu.make_async_copy(bwo_hbm, bwo, w_sem.at[5]),
    ]

    awk_copy.start()
    awq_copy.start()
    x_copy(0).start()
    awk_copy.wait()
    awqkT[D:, :] = _transposed(awqkv[:, D:2 * D])
    awq_copy.wait()
    for j in range(1, NBLK):
        x_copy(j).start()
    awqkT[0:D, :] = _transposed(awqkv[:, 0:D])
    x_copy(0).wait()
    for copy in late_copies:
        copy.start()

    def sub_rows(j):
        return [_span(j * NSUB + u, TB) for u in range(NSUB)]

    def next_block(j):
        return jnp.minimum(j + 1, NBLK - 1)

    def stream(layer, r):
        return jnp.where(layer == 0, io[r, :].astype(F32), xs[r, :])

    def a_norm(layer, j):
        r = _span(j, BLK)
        xns[r, :] = _layernorm(stream(layer, r))

    def a_proj(layer, j):
        rows = sub_rows(j)

        def q_part(r):
            pqT[:, r] = _phi(_dot(awqkT[0:D, :], xns[r, :], NT)).astype(BF16)
        pk = jnp.concatenate([_phi(_dot(awqkT[D:, :], xns[r, :], NT)) for r in rows], axis=1)
        a_norm(layer, next_block(j))
        for r in rows[:-1]:
            q_part(r)
        z = z_acc[...]
        for t in range(BLK // LANES):
            z = z + pk[:, _tile(t)]
        z_acc[...] = z
        g_acc[...] += _dot(pk, jnp.concatenate([xns[r, :] for r in rows], axis=0))
        q_part(rows[-1])

    def a_reduce():
        z = jnp.sum(z_acc[...].T, axis=0, keepdims=True)
        zh[...] = jnp.where(_head_of(_iota((H, D), 1)) == _iota((H, D), 0), z, 0.0)
        m_acc[...] = jnp.zeros_like(m_acc)
        for e in range(ND):
            lo, hi = _band(e)
            r = _iota((hi - lo, LANES), 0) + lo
            c = _iota((hi - lo, LANES), 1) + e * LANES
            kv = _dot(g_acc[lo:hi, :], awqkv[:, _tile(2 * ND + e)])
            kv = jnp.where(_head_of(r) == _head_of(c), kv, 0.0)
            m_acc[lo:hi, :] += _dot(kv, awo[_tile(e), :])
        mw[...] = m_acc[...].astype(BF16)

    def a_ratio(j):
        p = pqT[:, _span(j, BLK)]
        inv = 1.0 / (_dot(zh[...], p) + 1e-6)
        low = _iota((8, BLK), 0) < 4
        parts = []
        for h in range(0, H, 2):
            a = jnp.broadcast_to(inv[h:h + 1], (8, BLK))
            b = jnp.broadcast_to(inv[h + 1:h + 2], (8, BLK))
            parts += [a, a, jnp.where(low, a, b), b, b]
        return (p.astype(F32) * jnp.concatenate(parts, axis=0)).T.astype(BF16)

    def b_proj(r, xb):
        xn = _layernorm(xb)
        k = _dot(xn, bwqkv[:, D:2 * D]).astype(BF16)
        for t in range(ND):
            ks[t, r, :] = k[:, _tile(t)]
        upper = _iota((TB, LANES), 1) >= HALF
        for t in range(ND - 1):
            ks[ND + t, r, :] = jnp.where(upper, k[:, _tile(t)], k[:, _tile(t + 1)])
        qv = _dot(bwqvT[...], xn, NT)
        for t in range(ND):
            qs[t, :, r] = (qv[_tile(t), :] * Q_SCALE).astype(BF16)
        vts[:, r] = qv[D:, :]

    def a_out_b_proj(layer, j):
        rows = sub_rows(j)
        ratio = a_ratio(next_block(j))
        xbs = []
        for r in rows:
            xb = stream(layer, r) + _dot(xns[r, :], mw[...])
            xs[r, :] = xb
            xbs.append(xb)
        xns[_span(next_block(j), BLK), :] = ratio
        for r, xb in zip(rows, xbs):
            b_proj(r, xb)

    def head_q(h, cols):
        tile = (h * DH) // LANES
        off = h * DH - tile * LANES
        cross = jnp.where(off + DH > LANES, 1, 0)
        q = jnp.concatenate([qs[tile + cross, 0:HALF, cols], qs[tile, HALF:, cols]], axis=0)
        mine = ((_iota((LANES, BLK), 0) - off) & (LANES - 1)) < DH
        return tile + ND * cross, jnp.where(mine, q.astype(F32), 0.0).astype(BF16)

    def v_window(h):
        r0 = pl.multiple_of((h * DH) // 8 * 8, 8)
        return r0, h * DH - r0

    def load_v(h):
        r0, o0 = v_window(h)
        r = _iota((VW, S), 0)
        vm[...] = jnp.where((r >= o0) & (r < o0 + DH), vts[pl.ds(r0, VW), :], 1.0)

    def attn_tile(h_qk, h_pv, t):
        cols = _span(t, BLK)
        if h_qk is not None:
            kt, q = head_q(h_qk, cols)
        if h_pv is not None:
            m_old = m_scr[0:1, cols]
        m = acc = None
        for c in range(S // CK):
            keys = slice(c * CK, (c + 1) * CK)
            if h_qk is not None:
                st = _dot(ks[kt, keys, :], q)
            if h_pv is not None:
                old = s_scr[t, keys, :]
            if h_qk is not None:
                s_scr[t, keys, :] = st
                mm = jnp.max(st.reshape(CK // 8, 8, BLK), axis=0)
                m = mm if m is None else jnp.maximum(m, mm)
            if h_pv is not None:
                o = _dot(vm[:, keys], jnp.exp2(old - m_old).astype(BF16))
                acc = o if acc is None else acc + o
        if h_pv is not None:
            r0, o0 = v_window(h_pv)
            den = jnp.where(o0 == 0, acc[VW - 1:VW, :], acc[0:1, :])
            win = pl.ds(r0, VW)
            ots[win, cols] = jnp.where(_iota((VW, BLK), 0) >= o0, acc / den, ots[win, cols])
        if h_qk is not None:
            m_scr[:, cols] = jnp.broadcast_to(jnp.max(m, axis=0, keepdims=True), (8, BLK))

    def head_step(h):
        load_v(h - 1)
        for t in range(NBLK):
            attn_tile(h, h - 1, t)

    def b_out(j):
        r = _span(j, BLK)

        def part(lo, hi):
            return _dot(ots[lo:hi, r].astype(BF16), bwo[lo:hi, :], TN)
        xb = xs[r, :] + part(0, 2 * LANES)
        attn_tile(None, H - 1, j)
        xb = xb + part(2 * LANES, 4 * LANES)
        xb = xb + part(4 * LANES, D)
        xs[r, :] = xb
        io[r, :] = xb.astype(io.dtype)

    def layer_pair(layer):
        z_acc[...] = jnp.zeros_like(z_acc)
        g_acc[...] = jnp.zeros_like(g_acc)
        a_norm(layer, 0)

        def a_block(j):
            @pl.when(jnp.logical_and(layer == 0, j + 1 < NBLK))
            def _():
                x_copy(next_block(j)).wait()
            a_proj(layer, j)
        _loop(0, NBLK, a_block)

        @pl.when(layer == 0)
        def _():
            for copy in late_copies:
                copy.wait()

        a_reduce()
        xns[0:BLK, :] = a_ratio(0)
        bwqvT[0:D, :] = _transposed(bwqkv[:, 0:D])
        bwqvT[D:, :] = _transposed(bwqkv[:, 2 * D:3 * D])
        _loop(0, NBLK, lambda j: a_out_b_proj(layer, j))

        def first_head(i):
            attn_tile(0, None, 2 * i)
            attn_tile(0, None, 2 * i + 1)
        _loop(0, NBLK // 2, first_head)
        head_step(1)

        def head_pair(i):
            head_step(2 * i)
            head_step(2 * i + 1)
        _loop(1, H // 2, head_pair)

        load_v(H - 1)

        def out_block(j):
            b_out(j)

            @pl.when(layer == 1)
            def _():
                out_copy(j).start()
        _loop(0, NBLK, out_block)

    _loop(0, 2, layer_pair)
    for j in range(NBLK):
        out_copy(j).wait()


@jax.jit
def pallas_interleave_layers__linear_attn_block__mha_block__prompt_kernel(
    A_x: jax.Array,
    A_wqkv: jax.Array,
    A_wo: jax.Array,
    B_x: jax.Array,
    B_wqkv: jax.Array,
    B_wo: jax.Array,
):
    del B_x
    out = pl.pallas_call(
        _kernel,
        out_shape=jax.ShapeDtypeStruct((S, D), A_x.dtype),
        in_specs=[pl.BlockSpec(memory_space=pl.ANY)] * 5,
        out_specs=pl.BlockSpec(memory_space=pl.ANY),
        scratch_shapes=[
            pltpu.VMEM((S, D), A_x.dtype),
            pltpu.VMEM((D, 3 * D), A_wqkv.dtype),
            pltpu.VMEM((D, D), A_wo.dtype),
            pltpu.VMEM((D, 3 * D), B_wqkv.dtype),
            pltpu.VMEM((D, D), B_wo.dtype),
            pltpu.SemaphoreType.DMA((NBLK,)),
            pltpu.SemaphoreType.DMA((6,)),
            pltpu.VMEM((S, D), F32),
            pltpu.VMEM((S, D), BF16),
            pltpu.VMEM((2 * D, D), BF16),
            pltpu.VMEM((2 * D, D), BF16),
            pltpu.VMEM((D, S), BF16),
            pltpu.VMEM((D, D), F32),
            pltpu.VMEM((D, LANES), F32),
            pltpu.VMEM((D, D), F32),
            pltpu.VMEM((D, D), BF16),
            pltpu.VMEM((H, D), F32),
            pltpu.VMEM((2 * ND - 1, S, LANES), BF16),
            pltpu.VMEM((ND, LANES, S), BF16),
            pltpu.VMEM((D, S), F32),
            pltpu.VMEM((D, S), F32),
            pltpu.VMEM((NBLK, S, BLK), F32),
            pltpu.VMEM((8, S), F32),
            pltpu.VMEM((VW, S), F32),
        ],
        compiler_params=pltpu.CompilerParams(vmem_limit_bytes=100 * 1024 * 1024),
    )(A_x.reshape(S, D), A_wqkv, A_wo, B_wqkv, B_wo)
    return out.reshape(A_x.shape)
```
